```python
import os as _os
_os.environ.setdefault('JAX_PLATFORMS', 'cpu')
import jax
import jax.numpy as jnp

def _softmax(x, axis=-1):
    return jax.nn.softmax(x, axis=axis)

def _gelu(x):
    return jax.nn.gelu(x, approximate=True)

def _silu(x):
    return jax.nn.silu(x)

def _sigmoid(x):
    return jax.nn.sigmoid(x)

def _layernorm(x, axis=-1, eps=1e-05):
    m = jnp.mean(x, axis=axis, keepdims=True)
    v = jnp.var(x, axis=axis, keepdims=True)
    return (x - m) / jnp.sqrt(v + eps)

def _scatter_add(tgt, idx, src, axis=0):
    return tgt.at[idx].add(src)

def _segment_sum(src, seg, n):
    return jax.ops.segment_sum(src, seg, n)

class _Rng:

    def __init__(self, key):
        self._k = key

    def _next(self):
        self._k, sub = jax.random.split(self._k)
        return sub

    def normal(self, shape):
        return jax.random.normal(self._next(), shape, dtype=jnp.bfloat16)

    def randint(self, lo, hi, shape):
        return jax.random.randint(self._next(), shape, lo, hi, dtype=jnp.int32)

    def uniform(self, shape, lo=0.0, hi=1.0):
        return jax.random.uniform(self._next(), shape, jnp.bfloat16, lo, hi)

    def permutation(self, n):
        return jax.random.permutation(self._next(), n)
kernel_name = 'adaLN_cond__sliding_local_dilated__dense_activation_gelu__prompt'

def setup_inputs():
    _rng = _Rng(jax.random.key(int.from_bytes(__import__("os").urandom(4), "little")))
    _w = lambda a: (lambda t: t.astype(jnp.bfloat16) if jnp.issubdtype(t.dtype, jnp.floating) else t)(jnp.asarray(a))

    def _A_setup():
        B, S, D = (1, 2048, 576)
        return {'x': _w((lambda *s: _rng.normal(s) * 0.05)(B, S, D)), 'wqkv': _w((lambda *s: _rng.normal(s) * 0.05)(D, 3 * D)), 'wo': _w((lambda *s: _rng.normal(s) * 0.05)(D, D))}
    _A_in = _A_setup()

    def _B_setup():
        B, S, D, F = (1, 2048, 576, 4608)
        return {'x': _w((lambda *s: _rng.normal(s) * 0.05)(B, S, D)), 'w1': _w((lambda *s: _rng.normal(s) * 0.8)(D, F) * D ** (-0.5)), 'b1': _w((lambda *s: _rng.normal(s) * 0.8)(F) * 0.01), 'w2': _w((lambda *s: _rng.normal(s) * 0.8)(F, D) * F ** (-0.5)), 'b2': _w((lambda *s: _rng.normal(s) * 0.8)(D) * 0.01)}
    _B_in = _B_setup()
    return {'A_x': _A_in['x'], 'A_wqkv': _A_in['wqkv'], 'A_wo': _A_in['wo'], 'B_x': _B_in['x'], 'B_w1': _B_in['w1'], 'B_b1': _B_in['b1'], 'B_w2': _B_in['w2'], 'B_b2': _B_in['b2'], 'c': _w((lambda *s: _rng.normal(s) * 0.05)(1, 576) * 8.0), 'w_mod': _w((lambda *s: _rng.normal(s) * 0.05)(576, 6 * 576) * 576 ** (-0.5) * 8.0)}

def reference(A_x, A_wqkv, A_wo, B_x, B_w1, B_b1, B_w2, B_b2, c, w_mod):

    def _A_ref(x, wqkv, wo):
        B, S, D = x.shape
        H = 32
        Dh = D // H
        W, dil = (8, 2)
        qkv = (lambda x, *d: x.transpose(*d))((x @ wqkv).reshape(B, S, 3, H, Dh), 2, 0, 3, 1, 4)
        q, k, v = (qkv[0], qkv[1], qkv[2])
        scale = Dh ** (-0.5)
        pos = jnp.arange(S)
        off = jnp.arange(W) * dil
        idx = pos[:, None] - off[None, :]
        mask = idx >= 0
        idx_c = jnp.where(mask, idx, 0).reshape(-1)
        kg = k[:, :, idx_c, :].reshape(B, H, S, W, Dh)
        vg = v[:, :, idx_c, :].reshape(B, H, S, W, Dh)
        logits = jnp.einsum('bhsd,bhswd->bhsw', q, kg) * scale
        logits = jnp.where(mask[None, None, :, :], logits, -1000000000.0)
        attn = _softmax(logits, axis=-1)
        o = jnp.einsum('bhsw,bhswd->bhsd', attn, vg)
        return (lambda x, *d: x.transpose(*d))(o, 0, 2, 1, 3).reshape(B, S, D) @ wo

    def _B_ref(x, w1, b1, w2, b2):
        h = jnp.einsum('bsd,df->bsf', x, w1) + b1
        h = _gelu(h)
        return jnp.einsum('bsf,fd->bsd', h, w2) + b2
    x = A_x
    mod = (_silu(c) @ w_mod).reshape(c.shape[0], 6, 1, -1)
    sa, ca, ga, sb, cb, gb = (mod[:, 0].copy(), mod[:, 1].copy(), mod[:, 2].copy(), mod[:, 3].copy(), mod[:, 4].copy(), mod[:, 5].copy())
    h = _layernorm(x, axis=-1) * (1 + ca) + sa
    x = x + ga * _A_ref(h, A_wqkv, A_wo)
    h = _layernorm(x, axis=-1) * (1 + cb) + sb
    x = x + gb * _B_ref(h, B_w1, B_b1, B_w2, B_b2)
    return x
```

```python
import jax
import jax.numpy as jnp
from jax import lax
import jax.experimental.pallas as pl
import jax.experimental.pallas.tpu as pltpu

F32, BF16, U32 = jnp.float32, jnp.bfloat16, jnp.uint32

S, D, F = 2048, 576, 4608
DH = 18
WIN, DIL = 8, 2
EPS = 1e-5
LOG2E = 1.4426950408889634
L = 128
NT = S // L
NU = NT // 2
NB = NT // 4
OCT = 8 * DH
KS = 512
FC = 512
NC = F // FC
GROUPS = (1, 4, 0, 3, 6, 2, 5)
EARLY = 2
WQ_PARTS = ((0, 384), (384, 256), (640, 512), (1152, 576))


def _op_a(a11, a12, a21, a22):
    return [a11 + a22, a21 + a22, a11, a22, a11 + a12, a11 - a21, a12 - a22]


def _op_b(b11, b12, b21, b22):
    return [b11 - b22, b11, b22 - b12, b21 - b11, b22, b11 - b12, b21 - b22]


def _op2(op, get, r):
    terms = (((0, 0), (1, 1)), ((1, 0), (1, 1)), ((0, 0),), ((1, 1),), ((0, 0), (0, 1)),
             ((0, 0), (1, 0)), ((0, 1), (1, 1))) if op is _op_a else (
             ((0, 0), (1, 1)), ((0, 0),), ((1, 1), (0, 1)), ((1, 0), (0, 0)), ((1, 1),),
             ((0, 0), (0, 1)), ((1, 0), (1, 1)))

    def outer(i, j):
        v = [get(2 * a + i, 2 * b + j) for a, b in terms[r]]
        if len(v) == 1:
            return v[0]
        return v[0] + v[1] if op is _op_a and r < 5 else v[0] - v[1]

    return op(outer(0, 0), outer(0, 1), outer(1, 0), outer(1, 1))


def _combine(prod, fin):
    m2 = prod(1)
    m4 = prod(3)
    fin(1, 0, m2 + m4)
    m5 = prod(4)
    m3 = prod(2)
    fin(0, 1, m5 - m3)
    m1 = prod(0)
    fin(0, 0, ((m4 + m5) + m1) + prod(6))
    fin(1, 1, ((m2 - m3) - m1) + prod(5))


def _combine2(prod, fin):
    m = {}

    def outer(r, oi=None, oj=None, fn=None):
        def inner_fin(i, j, v):
            m[r, i, j] = v
            if fn is not None:
                fin(2 * oi + i, 2 * oj + j, fn(lambda k: m[k, i, j]))

        _combine(lambda q: prod(7 * r + q), inner_fin)

    outer(1)
    outer(3, 1, 0, lambda g: g(1) + g(3))
    outer(4)
    outer(2, 0, 1, lambda g: g(4) - g(2))
    outer(0)
    outer(6, 0, 0, lambda g: ((g(3) + g(4)) + g(0)) + g(6))
    outer(5, 1, 1, lambda g: ((g(1) - g(2)) - g(0)) + g(5))


def _ld(ref, *idx):
    return pltpu.bitcast(ref.bitcast(U32)[idx], BF16)


def _mm(a, b):
    return jnp.dot(a, b, preferred_element_type=F32)


GELU_C0 = 0.7978845608028654
GELU_IN = (GELU_C0 * 0.044715) ** (1.0 / 3.0)
GELU_OUT = 0.5 / GELU_IN


def _gelu(y):
    return y * (1.0 + jnp.tanh(y * (y * y + GELU_C0 / GELU_IN)))


def _lo(u):
    return lax.bitcast_convert_type(u << 16, F32)


def _hi(u):
    return lax.bitcast_convert_type(u & jnp.uint32(0xFFFF0000), F32)


def _kernel(x_hbm, wqkv_hbm, wo_hbm, w1_hbm, b1_hbm, w2_hbm, b2_hbm, c_hbm, wm_hbm,
            out_hbm,
            xv, wqkv_v, wo_v, w1_v, w2_v,
            s_col, modt, tq, two, wo_t, wq_s, wo_s, w1_s, w2_s, h2_s, acc, ob,
            st1, st2, hop, qkv, logit, h2_f, v_head, prob, att, aop, x1_s, tw, act,
            wm_v, b1_v, b2_v, c_v, s_row, sem, out_sem, zeros):
    @pl.loop(0, 2)
    def _(i):
        zeros[i] = 0

    zero = zeros[0]
    uses = [0]

    def fresh():
        uses[0] += 1
        return zero * uses[0]

    tasks, stats, issued = [], [], [0]

    def spawn(gen, queue=tasks):
        next(gen)
        queue.append(gen)

    def step(queue, token):
        if queue:
            try:
                queue[0].send(token)
            except StopIteration:
                queue.pop(0)

    def drain(queue=tasks):
        while queue:
            step(queue, None)

    def run(gen):
        for _ in gen:
            pass

    def gate(ref, slot, token):
        if token is not None:
            if ref.dtype == BF16:
                ref[slot, pl.ds(0, 16), pl.ds(0, L)] = token[:16].astype(BF16)
            else:
                ref[slot, pl.ds(0, 8), pl.ds(0, L)] = lax.bitcast_convert_type(token[:8], ref.dtype)

    copies = {}

    def dma(name, src, dst):
        group = copies.setdefault(name, [])
        group.append(pltpu.make_async_copy(src, dst, sem.at[list(copies).index(name)]))

    def wait(*names):
        for cp in [cp for n in names for cp in copies[n]]:
            cp.wait()

    def fetch_x(name, u):
        dma(name, x_hbm.at[:, pl.ds(2 * L * u, 2 * L)], xv.at[u])

    def fetch_wqkv(name, i):
        dma(name, wqkv_hbm.at[:, pl.ds(*WQ_PARTS[i])], wqkv_v[i].at[0])

    def fetch_wm(name, lo, hi):
        cols = pl.ds(L * lo, L * (hi - lo))
        dma(name, wm_hbm.at[:, cols], wm_v.at[:, cols])

    def fetch_w1(name, i):
        dma(name, w1_hbm.at[:, pl.ds(FC * i, FC)], w1_v.at[i, pl.ds(0, D)])

    dma("vectors", c_hbm, c_v)
    dma("vectors", b1_hbm, b1_v)
    dma("vectors", b2_hbm, b2_v)
    fetch_wqkv("q a", 0)
    fetch_wm("shift", 0, 5)
    fetch_wm("scale", 5, 9)
    fetch_x("x", 0)
    fetch_wqkv("q b", 1)
    fetch_x("x b", 1)
    fetch_wqkv("k", 2)
    fetch_x("v", 2)
    fetch_wqkv("v", 3)
    dma("wo", wo_hbm, wo_v.at[0])
    fetch_x("wo", 3)
    fetch_wm("mod b", 9, 14)
    fetch_w1("w1", 0)
    fetch_wm("mod c", 14, 23)
    for u in range(4, NU):
        fetch_x("x rest", u)
    fetch_wm("w2", 23, 27)
    for i in range(NC):
        dma("w2", w2_hbm.at[:, pl.ds(FC * i, FC)], w2_v.at[i])
    for i in range(1, NC):
        fetch_w1("w1 rest", i)

    def mod_vec(z, i, r0, n):
        return modt[i // 2][z, pl.ds(D * (i % 2) + r0, n), :]

    def fold(v):
        parts = [v[r0:r0 + 8] for r0 in range(0, v.shape[0], 8)]
        while len(parts) > 1:
            parts = [a + b for a, b in zip(parts[::2], parts[1::2])] + parts[len(parts) // 2 * 2:]
        return parts[0]

    def store_mod(j, row):
        col = lax.broadcasted_iota(jnp.int32, row.shape, 1) + L * j
        row = jnp.where(((col >= D) & (col < 2 * D)) | ((col >= 4 * D) & (col < 5 * D)), 1.0 + row, row)
        row = row * jnp.where(col >= 5 * D, GELU_OUT, jnp.where(col >= 3 * D, GELU_IN, 1.0))
        modt[j // 9][0, pl.ds(L * (j % 9), L), :] = jnp.broadcast_to(row, (L, L)).T

    def mod_tiles(lo, hi):
        for j in range(lo, hi):
            store_mod(j, _mm(s_row[fresh()], wm_v[:, pl.ds(L * j, L)])[:1])

    def mod_tiles_vpu(lo, hi):
        for j in range(lo, hi):
            s = None
            for r0 in range(0, D, 96):
                token = yield
                gate(s_col, 1, token if token is None or s is None else token[:8] + s)
                v = fold(wm_v[pl.ds(r0, 96), pl.ds(L * j, L)].astype(F32) * s_col[fresh(), pl.ds(r0, 96), :])
                s = v if s is None else s + v
            store_mod(j, jnp.sum(s, axis=0, keepdims=True))

    def ln_finish(dst, t, pivot, s1, s2):
        m = jnp.sum(s1, axis=0, keepdims=True) * (1.0 / D)
        var = jnp.sum(s2, axis=0, keepdims=True) * (1.0 / D) - m * m
        r = lax.rsqrt(jnp.maximum(var, 0.0) + EPS)
        dst[t, 0] = jnp.broadcast_to(r, (16, L))
        dst[t, 1] = jnp.broadcast_to((pivot + m) * r, (16, L))

    def pad_k(a):
        return jnp.concatenate([a, jnp.zeros((L - a.shape[0], a.shape[1]), a.dtype)], axis=0)

    def store_one_level(dst, strip, release):
        for s in range(OCT // 16):
            rows = pl.ds(16 * s, 16)
            for kk in range(2):
                release((yield))
                ops = _op_a(strip(0, kk, s), strip(0, 2 + kk, s), strip(1, kk, s), strip(1, 2 + kk, s))
                for r, v in enumerate(ops):
                    dst[0, 2 * r + kk, rows, :] = v.astype(BF16)
                dst[0, 14 + kk, rows, :] = strip(kk, 4, s).astype(BF16)

    def head_major(src, kt, row0, dp):
        u = src[kt, pl.ds(row0 // 2 + dp, 8, stride=DH // 2), :]
        return jnp.concatenate([_lo(u), _hi(u)], axis=0)

    def transpose_wqkv(part):
        s0, n = WQ_PARTS[part]
        for kt in range(5):
            gate(wqkv_v[part], 1, (yield))
            blk = wqkv_v[part][fresh(), pl.ds(L * kt, min(L, D - L * kt)), :]
            if kt == 4:
                blk = pad_k(blk)
            tq[kt, pl.ds(s0 // 2, n // 2), :] = pltpu.bitcast(blk.T, U32)

    def prep_wqkv(ch):
        z = fresh()
        return store_one_level(wq_s[ch], lambda i, kt, s: head_major(tq, kt + z, OCT * (2 * ch + i), s),
                               lambda token: gate(tq, 5, token))

    def prep_wo():
        for nt in range(5):
            for r0 in range(0, D, 192):
                gate(wo_v, 1, (yield))
                w = min(L, D - L * nt)
                u = pltpu.bitcast(wo_v[fresh(), pl.ds(r0, 192), pl.ds(L * nt, w)], U32)
                if w < L:
                    u = jnp.concatenate([u, jnp.zeros((96, L - w), U32)], axis=1)
                two[nt, pl.ds(r0 // 2, 96), :] = u
        for nt in range(5):
            for kt in range(5):
                gate(two, 5, (yield))
                z = fresh()
                p = [head_major(two, nt + z, OCT * (s // 9), s % 9) if s < D // 16 else jnp.zeros((16, L), F32)
                     for s in range(8 * kt, 8 * kt + 8)]
                wo_t[kt, pl.ds(L * nt, L), :] = jnp.concatenate(p, axis=0).astype(BF16).T
        for ch in range(2):
            z = fresh()
            yield from store_one_level(
                wo_s[ch], lambda i, kt, s: wo_t[kt + z, pl.ds(OCT * (ch + 2 * i) + 16 * s, 16), :].astype(F32),
                lambda token: gate(wo_t, 5, token))

    def place_biases():
        modt[3][0] = jnp.broadcast_to(b2_v[...].astype(F32).reshape(1, D) * (1.0 / GELU_OUT), (L, D)).T
        b1 = jnp.broadcast_to(b1_v[...].astype(F32).reshape(1, F), (16, F))
        b1 = jnp.where(lax.broadcasted_iota(jnp.int32, b1.shape, 0) < 2, b1, 0.0).astype(BF16)
        for i in range(NC):
            w1_v[i, pl.ds(D, 16), :] = b1[:, FC * i:FC * i + FC]

    def transpose_w1(p):
        for k in range(5):
            gate(w1_v, NC, (yield))
            tw[k] = pltpu.bitcast(w1_v[p + fresh(), pl.ds(L * k, L), :].T, U32)

    def prep_w1(strips):
        for s in strips:
            def at(start, n):
                return pl.ds(start if isinstance(start, int) else pl.multiple_of(start, n), n)

            for r in range(7):
                gate(tw, 5, (yield))
                z = fresh()

                def get(i, k):
                    return pltpu.bitcast(tw[z + k, at(L * (3 - i) // 2 + 8 * s, 8), :], BF16)

                for q, v in enumerate(_op2(_op_a, lambda i, k: get(i, k).astype(F32), r)):
                    w1_s[0, 7 * r + q, at(16 * s, 16), :] = v.astype(BF16)
                if r < 4:
                    w1_s[0, 49 + r, at(16 * s, 16), :] = get(r, 4)

    def prep_w2(p, r):
        for s0 in range(0, OCT, 16):
            gate(w2_v, NC, (yield))
            src = p + fresh()
            ops = _op2(_op_a, lambda i, k: w2_v[src, pl.ds(OCT * i + s0, 16), pl.ds(L * k, L)].astype(F32), r)
            for q, v in enumerate(ops):
                w2_s[r][0, q, pl.ds(s0, 16), :] = v.astype(BF16)

    def store_operands(dst, slot, strip, release=lambda token: None):
        for r0 in range(0, KS // 2, 16):
            release((yield))
            ops = _op_b(strip(0, r0), strip(1, r0), strip(0, KS // 2 + r0), strip(1, KS // 2 + r0))
            for r, v in enumerate(ops):
                dst[slot, 2 * r + r0 // L, pl.ds(r0 % L, 16), :] = v.astype(BF16)
        for j in range(2):
            release((yield))
            for r0 in range(KS, D, 16):
                dst[slot, 14 + j, pl.ds(r0 - KS, 16), :] = strip(j, r0).astype(BF16)

    def mm(a, b):
        d = _mm(a, b)
        first = 32 * (issued[0] % 4)
        issued[0] += 1
        step(tasks, d[first:])
        step(stats, d[first + 16:])
        return d

    def project(w_ref, b_ref, slot, fin):
        z = fresh()
        _combine(lambda r: (mm(_ld(w_ref, z, 2 * r), _ld(b_ref, slot + z, 2 * r))
                            + mm(_ld(w_ref, z, 2 * r + 1), _ld(b_ref, slot + z, 2 * r + 1))),
                 lambda i, j, v: fin(i, j, v + mm(_ld(w_ref, z, 14 + i), _ld(b_ref, slot + z, 14 + j))))

    def x_rows(u, j, r0, n):
        return xv[u, pl.ds(r0, n), pl.ds(L * j, L)].astype(F32)

    def ln1_stats(u):
        def steps():
            for j in range(2):
                for r0 in range(0, D, 48):
                    token = yield
                    if token is not None and r0:
                        token = jnp.concatenate([token[:8] + s1, s2], axis=0)
                    gate(xv, NU, token)
                    x = x_rows(u + fresh(), j, r0, 48)
                    if not r0:
                        pivot = x[:1]
                    d = x - pivot
                    s1, s2 = (s1 + fold(d), s2 + fold(d * d)) if r0 else (fold(d), fold(d * d))
                ln_finish(st1, 2 * u + j, pivot, s1, s2)

        spawn(steps(), queue=stats)

    def hop_slot(u):
        return (hop[0], 0) if isinstance(u, int) and u == 0 else (hop[1], u - 1)

    def ln1_operands(u):
        z = fresh()
        spawn(store_operands(*hop_slot(u), lambda j, r0: (
            (x_rows(u + z, j, r0, 16) * st1[2 * u + j + z, 0] - st1[2 * u + j + z, 1]) * mod_vec(z, 1, r0, 16)
            + mod_vec(z, 0, r0, 16)), lambda token: gate(st1.at[NT], 0, token)))

    def proj_qkv(u, ty, halves=(0, 1)):
        for op in halves:
            def fin(i, j, v):
                qkv[ty][2 * op + i][j][u, pl.ds(0, OCT), :] = v
            project(wq_s[2 * ty + op], *hop_slot(u), fin)

    def lane(x):
        return lax.broadcasted_iota(jnp.int32, x.shape, 1)

    def back(cur, prev, s):
        if prev is not None:
            cur = jnp.where(lane(cur) >= L - s, prev, cur)
        return pltpu.roll(cur, s, 1)

    def ahead(cur, nxt, s):
        if nxt is not None:
            cur = jnp.where(lane(cur) < s, nxt, cur)
        return pltpu.roll(cur, L - s, 1)

    def tile(bufs, z, u, dt, idx):
        if isinstance(u, int) and not 0 <= 2 * u + dt < NT:
            return None
        return bufs[dt % 2][u + z + dt // 2, idx]

    def is_first(u, dt):
        return isinstance(u, int) and 2 * u + dt == 0

    HALF = WIN // 2
    FAR = HALF * DIL
    DS, DV = 3, 2

    def attention_probs(u, dts):
        def softmax(dt, o):
            z, head = fresh(), is_first(u, dt)
            lg = [logit[dt % 2 + z, o, w] for w in range(WIN)]
            for w in range(HALF, WIN):
                lg[w] = back(lg[w], None if head else logit[(dt - 1) % 2 + z, o, w], FAR)
            if head:
                lg = [jnp.where(lane(v) >= DIL * w, v, -1e9 * DH ** 0.5) for w, v in enumerate(lg)]
            m = lg[0]
            for v in lg[1:]:
                m = jnp.maximum(m, v)
            e = [jnp.exp2((v - m) * (LOG2E * DH ** -0.5)) for v in lg]
            inv = 1.0 / (((e[0] + e[1]) + (e[2] + e[3])) + ((e[4] + e[5]) + (e[6] + e[7])))
            for w in range(WIN):
                prob[o][dt % 2][u + dt // 2, w] = e[w] * inv

        done = None
        for dt in dts:
            z = fresh()
            for o in range(4):
                near, far = [None] * HALF, [None] * HALF
                for d in range(0, DH, DS):
                    rows = pl.ds(8 * d, 8 * DS)
                    q, k = tile(qkv[0][o], z, u, dt, rows), tile(qkv[1][o], z, u, dt, rows)
                    k_prev = tile(qkv[1][o], z, u, dt - 1, rows)
                    qa = ahead(q, tile(qkv[0][o], z, u, dt + 1, rows), FAR)
                    for w in range(HALF):
                        ks = back(k, k_prev, DIL * w) if w else k
                        near[w] = near[w] + fold(q * ks) if d else fold(q * ks)
                        far[w] = far[w] + fold(qa * ks) if d else fold(qa * ks)
                    if d == 9 and done is not None:
                        softmax(*done)
                for w in range(HALF):
                    logit[dt % 2 + z, o, w] = near[w]
                    logit[dt % 2 + z, o, HALF + w] = far[w]
                done = (dt, o)
        softmax(*done)

    def first_values():
        for o in range(4):
            v_head[0, o] = jnp.broadcast_to(qkv[2][o][0][fresh(), pl.ds(0, OCT), :][:, 0:1], (OCT, L))

    def attention_values(u):
        for dt in range(2):
            z, head = fresh(), is_first(u, dt)
            for o in range(4):
                p = [tile(prob[o], z, u, dt, w) for w in range(WIN)]
                f = [ahead(p[HALF + w], tile(prob[o], z, u, dt + 1, HALF + w), FAR) for w in range(HALF)]
                if head:
                    lead = ahead((p[4] + p[5]) + (p[6] + p[7]), None, FAR)
                p, f = ([jnp.concatenate([a] * DV, axis=0) for a in wt[:HALF]] for wt in (p, f))
                for d in range(0, DH, DV):
                    rows = pl.ds(8 * d, 8 * DV)
                    v, v_prev = tile(qkv[2][o], z, u, dt, rows), tile(qkv[2][o], z, u, dt - 1, rows)
                    if head:
                        v_prev = v_head[z, o, rows, :]
                        att[o][1 + z, 1, 1, rows, :] = jnp.concatenate([lead] * DV, axis=0) * v_prev
                    vs = [v] + [back(v, v_prev, DIL * w) for w in range(1, HALF)]
                    for i, wt in enumerate((p, f)):
                        att[o][u % 2 + z, dt, i, rows, :] = (
                            (wt[0] * vs[0] + wt[1] * vs[1]) + (wt[2] * vs[2] + wt[3] * vs[3]))
        z = fresh()

        def strip(j, r0):
            buf, rows = att[r0 // OCT], pl.ds(r0 % OCT, 16)
            before = buf[u % 2 + z, 0, 1, rows, :] if j else buf[1 - u % 2 + z, 1, 1, rows, :]
            return buf[u % 2 + z, j, 0, rows, :] + back(buf[u % 2 + z, j, 1, rows, :], before, FAR)

        run(store_operands(aop, 0, strip))

    def proj_out(u):
        z, pivot, sums = fresh(), {}, [[], []]
        for ch in range(2):
            def fin(i, j, v):
                r0 = OCT * (ch + 2 * i)
                x1 = x_rows(u + z, j, r0, OCT) + mod_vec(z, 2, r0, OCT) * v
                x1_s[j][u, pl.ds(r0, OCT), :] = x1
                d = x1 - pivot.setdefault(j, x1[:1])
                s1, s2 = d[:8], d[:8] * d[:8]
                for k in range(8, OCT, 8):
                    s1, s2 = s1 + d[k:k + 8], s2 + d[k:k + 8] * d[k:k + 8]
                sums[j].append((s1, s2))
            project(wo_s[ch], aop, 0, fin)
        for j in range(2):
            ln_finish(st2, 2 * u + j, pivot[j], *[fold(jnp.concatenate(s, axis=0)) for s in zip(*sums[j])])

    def mlp_operands(b, half, paced=True):
        z = fresh()

        def rows(r0):
            return pl.ds(r0 if isinstance(r0, int) else pl.multiple_of(r0, 16), 16)

        def strip(j, r0):
            x1 = x1_s[j % 2][2 * b + j // 2 + z, rows(r0), :]
            return ((x1 * st2[4 * b + j + z, 0] - st2[4 * b + j + z, 1]) * modt[2][z, rows(r0), :]
                    + modt[1][z, rows(D + r0), :])

        for s in range(4):
            s0 = 64 * half + 16 * s
            if not paced:
                x = {(k, j): strip(j, L * k + s0) for k in range(4) for j in range(4)}
                for r in range(7):
                    for q, v in enumerate(_op2(_op_b, lambda k, j: x[k, j], r)):
                        h2_s[b, 7 * r + q, rows(s0), :] = v.astype(BF16)
                continue
            for k in range(4):
                token = yield
                for j in range(2):
                    gate(x1_s[j], NU, token)
                for j in range(4):
                    h2_f[0, pl.ds(16 * (4 * k + j), 16), :] = strip(j, L * k + s0)
            for r in range(7):
                gate(h2_f, 1, (yield))
                zz = fresh()
                for q, v in enumerate(_op2(_op_b, lambda k, j: h2_f[zz, pl.ds(16 * (4 * k + j), 16), :], r)):
                    h2_s[b, 7 * r + q, rows(s0), :] = v.astype(BF16)
        for s in range(2):
            s0 = 32 * half + 16 * s
            token = yield
            for j in range(2):
                gate(x1_s[j], NU, token)
            for j in range(4):
                h2_s[b, 49 + j, rows(s0), :] = strip(j, KS + s0).astype(BF16)

    def mlp_hidden(b):
        z, hid = fresh(), {}

        def fin(i, j, v):
            hid[3 - i, j] = _gelu(v + _mm(_ld(w1_s, z, 49 + i), _ld(h2_s, z + b, 49 + j)))

        def prod(r):
            return (mm if r // 7 in (1, 4, 0) else _mm)(_ld(w1_s, z, r), _ld(h2_s, z + b, r))

        _combine2(prod, fin)
        for r in range(7):
            for q, v in enumerate(_op2(_op_b, lambda k, j: hid[k, j], r)):
                act[r][b, q] = v.astype(BF16)

    def mlp_products(groups, started, nxt=None):
        z, issued[0] = fresh(), 0
        for r in groups:
            for q in range(7):
                w = _ld(w2_s[r], z, q)
                for b in range(NB):
                    d = mm(w, _ld(act[r], z + b, q))
                    if started is False:
                        acc[b, r, q] = d
                    elif started is True:
                        acc[b, r, q] += d
                    else:
                        acc[b, r, q] = jnp.where(started, acc[b, r, q], 0.0) + d
            if nxt is not None:
                spawn(prep_w2(nxt, r))

    def write_out(b, i, j):
        rows, col = pl.ds(D // 2 * i, D // 2), 4 * L * b + 2 * L * j
        col = col if isinstance(col, int) else pl.multiple_of(col, 2 * L)
        return pltpu.make_async_copy(ob.at[b, rows, pl.ds(2 * L * j, 2 * L)],
                                     out_hbm.at[rows, pl.ds(col, 2 * L)], out_sem)

    def mlp_finish(b):
        z = fresh()

        def prod(p):
            r, q = divmod(p, 7)
            if r in GROUPS[:EARLY]:
                return acc[b, r, q]
            return acc[b, r, q] + _mm(_ld(w2_s[r], z, q), _ld(act[r], b, q))

        def fin(i, j, v):
            rows, zz = pl.ds(OCT * i, OCT), fresh()
            v = mod_vec(zz, 5, OCT * i, OCT) * (v + mod_vec(zz, 6, OCT * i, OCT))
            ob[b, rows, pl.ds(L * j, L)] = (x1_s[j % 2][2 * b + j // 2, rows, :] + v).astype(BF16)
            if i % 2 and j % 2:
                write_out(b, i // 2, j // 2).start()

        _combine2(prod, fin)

    for group in copies.values():
        for cp in group:
            cp.start()
    for buf in (*hop, aop):
        buf[:, pl.ds(14, 2), pl.ds(D - KS, 5 * L - D), :] = jnp.zeros((buf.shape[0], 2, 5 * L - D, L), BF16)
    w1_v[pl.ds(0, NC), pl.ds(D + 16, 5 * L - D - 16), :] = jnp.zeros((NC, 5 * L - D - 16, FC), BF16)
    row = lax.broadcasted_iota(jnp.int32, (5 * L - D, L), 0)
    lead = round(GELU_IN * 256) / 256
    one = jnp.where(row == 0, lead, jnp.where(row == 1, GELU_IN - lead, 0.0)).astype(BF16)
    for b in range(NB):
        for j in range(4):
            h2_s[b, 49 + j, pl.ds(D - KS, 5 * L - D), :] = one
    for j in range(2):
        x1_s[j][1] = jnp.zeros((D, L), F32)
        st2[2 + j] = jnp.zeros((4, 16, L), F32)
    wait("vectors")
    place_biases()
    cf = c_v[...].astype(F32)
    silu = cf * (1.0 / (1.0 + jnp.exp(-cf)))
    s_row[0] = jnp.broadcast_to(silu, (16, D)).astype(BF16)
    s_col[0] = jnp.broadcast_to(silu, (L, D)).T
    wait("q a")
    run(transpose_wqkv(0))
    run(prep_wqkv(0))
    wait("shift")
    mod_tiles(0, 5)
    wait("scale")
    mod_tiles(5, 9)
    wait("x")
    ln1_stats(0)
    drain(stats)
    ln1_operands(0)
    drain()
    wait("q b")
    run(transpose_wqkv(1))
    spawn(prep_wqkv(1))
    proj_qkv(0, 0, (0,))
    drain()
    wait("x b")
    ln1_stats(1)
    drain(stats)
    ln1_operands(1)
    proj_qkv(0, 0, (1,))
    drain()
    wait("k")
    run(transpose_wqkv(2))
    spawn(prep_wqkv(2))
    spawn(prep_wqkv(3))
    proj_qkv(1, 0)
    drain()
    wait("v")
    ln1_stats(2)
    drain(stats)
    ln1_operands(2)
    proj_qkv(0, 1)
    drain()
    run(transpose_wqkv(3))
    spawn(prep_wqkv(4))
    spawn(prep_wqkv(5))
    attention_probs(0, (0,))
    proj_qkv(1, 1)
    wait("wo")
    drain()
    spawn(prep_wo())
    attention_probs(0, (1, 2))
    proj_qkv(0, 2)
    first_values()
    ln1_stats(3)
    proj_qkv(2, 0)
    wait("mod b")
    attention_values(0)
    proj_qkv(2, 1)
    drain()
    drain(stats)
    ln1_operands(3)
    wait("w1", "mod c")
    mod_tiles(9, 23)
    proj_out(0)
    run(transpose_w1(0))
    drain()

    def attention_step(u, carry):
        issued[0] = 0
        nxt, done, s = jnp.minimum(u + 3, NU - 1), jnp.maximum(u - 2, 0), 2 * jnp.minimum(u - 1, 3)
        ln1_stats(nxt)
        attention_probs(u, (1, 2))
        proj_qkv(u, 2)
        attention_values(u)
        proj_qkv(u + 2, 0)
        spawn(mlp_operands(lax.shift_right_logical(done, 1), lax.bitwise_and(done, 1)))
        proj_qkv(u + 2, 1)
        drain(stats)
        ln1_operands(nxt)
        spawn(prep_w1((s, s + 1)))
        proj_out(u)
        drain()
        return carry

    wait("x rest")
    lax.fori_loop(1, NU - 2, attention_step, None)

    issued[0] = 0
    wait("w2")
    run(mlp_operands(NB - 2, 0, paced=False))
    proj_qkv(NU - 1, 2)
    attention_probs(NU - 2, (1, 2, 3))
    for r in GROUPS[:EARLY]:
        spawn(prep_w2(0, r))
    proj_qkv(NU - 2, 2)
    mlp_hidden(0)
    attention_values(NU - 2)
    drain()
    proj_out(NU - 2)
    attention_values(NU - 1)
    spawn(mlp_operands(NB - 2, 1))
    proj_out(NU - 1)
    wait("w1 rest")
    drain()
    mlp_hidden(1)
    run(mlp_operands(NB - 1, 0, paced=False))
    mlp_hidden(2)
    run(mlp_operands(NB - 1, 1, paced=False))
    mlp_hidden(3)
    for r in GROUPS[EARLY:]:
        run(prep_w2(0, r))
    spawn(mod_tiles_vpu(23, 27), queue=stats)
    mlp_products(GROUPS[:EARLY], False)
    drain(stats)

    def mlp_step(c, carry):
        spawn(transpose_w1(c))
        spawn(prep_w1(range(8)))
        for r in GROUPS[:EARLY]:
            spawn(prep_w2(c, r))
        mlp_products(GROUPS[EARLY:], c > 1, c)
        late = tasks[:]
        assert len(late) <= len(GROUPS) - EARLY
        tasks.clear()
        for b in range(NB):
            mlp_hidden(b)
        tasks.extend(late)
        mlp_products(GROUPS[:EARLY], True)
        drain()
        return carry

    lax.fori_loop(1, NC, mlp_step, None)

    for b in range(NB):
        mlp_finish(b + fresh())
    for b in range(NB):
        for q in range(4):
            write_out(b, q // 2, q % 2).wait()


@jax.jit
def pallas_adaLN_cond__sliding_local_dilated__dense_activation_gelu__prompt_kernel(
    A_x: jax.Array,
    A_wqkv: jax.Array,
    A_wo: jax.Array,
    B_x: jax.Array,
    B_w1: jax.Array,
    B_b1: jax.Array,
    B_w2: jax.Array,
    B_b2: jax.Array,
    c: jax.Array,
    w_mod: jax.Array,
):
    del B_x
    vmem = pltpu.VMEM
    scratch = [
        vmem((NU + 1, D, 2 * L), BF16),
        [vmem((2, D, n), BF16) for _, n in WQ_PARTS],
        vmem((2, D, D), BF16),
        vmem((NC + 1, 5 * L, FC), BF16),
        vmem((NC + 1, D, FC), BF16),
        vmem((2, D, L), F32),
        [vmem((1, 2 * D, L), F32)] * 3 + [vmem((1, D, L), F32)],
        vmem((6, 896, L), U32),
        vmem((6, 320, L), U32),
        vmem((6, 5 * L, L), BF16),
        [vmem((1, 16, OCT, L), BF16)] * 6,
        [vmem((1, 16, OCT, L), BF16)] * 2,
        vmem((1, 53, L, L), BF16),
        [vmem((1, 8, OCT, L), BF16)] * 7,
        vmem((NB, 53, L, L), BF16),
        vmem((NB, 7, 8, OCT, L), F32),
        vmem((NB, D, 4 * L), BF16),
        vmem((NT + 1, 4, 16, L), F32),
        vmem((NT + 1, 4, 16, L), F32),
        [vmem((1, 16, L, L), BF16), vmem((NU - 1, 16, L, L), BF16)],
        [[[vmem((NU, 192, L), F32)] * 2] * 4] * 3,
        vmem((2, 4, WIN, 8, L), F32),
        vmem((2, 256, L), F32),
        vmem((1, 4, OCT, L), F32),
        [[vmem((NU, WIN, 8, L), F32)] * 2] * 4,
        [vmem((2, 2, 2, OCT, L), F32)] * 4,
        vmem((1, 16, L, L), BF16),
        [vmem((NU + 1, D, L), F32)] * 2,
        vmem((6, FC // 2, L), U32),
        [vmem((NB, 7, L, L), BF16)] * 7,
        vmem((D, 6 * D), BF16),
        vmem((F,), BF16),
        vmem((D,), BF16),
        vmem((1, D), BF16),
        vmem((1, 16, D), BF16),
        pltpu.SemaphoreType.DMA((16,)),
        pltpu.SemaphoreType.DMA,
        pltpu.SMEM((2,), jnp.int32),
    ]
    out_t = pl.pallas_call(
        _kernel,
        in_specs=[pl.BlockSpec(memory_space=pl.ANY)] * 9,
        out_specs=pl.BlockSpec(memory_space=pl.ANY),
        out_shape=jax.ShapeDtypeStruct((D, S), BF16),
        scratch_shapes=scratch,
        compiler_params=pltpu.CompilerParams(vmem_limit_bytes=120 * 1024 * 1024),
    )(A_x.reshape(S, D).T, A_wqkv, A_wo, B_w1, B_b1, B_w2.T, B_b2, c, w_mod)
    return out_t.T.reshape(1, S, D)
```
